```python
import os as _os
_os.environ.setdefault("JAX_PLATFORMS", "cpu")
import jax
import jax.numpy as jnp

def _softmax(x, axis=-1):
    return jax.nn.softmax(x, axis=axis)
def _gelu(x):
    return jax.nn.gelu(x, approximate=True)
def _silu(x):
    return jax.nn.silu(x)
def _sigmoid(x):
    return jax.nn.sigmoid(x)
def _layernorm(x, axis=-1, eps=1e-5):
    m = jnp.mean(x, axis=axis, keepdims=True)
    v = jnp.var(x, axis=axis, keepdims=True)
    return (x - m) / jnp.sqrt(v + eps)
def _scatter_add(tgt, idx, src, axis=0):
    return tgt.at[idx].add(src)
def _segment_sum(src, seg, n):
    return jax.ops.segment_sum(src, seg, n)
class _Rng:
    def __init__(self, key):
        self._k = key
    def _next(self):
        self._k, sub = jax.random.split(self._k)
        return sub
    def normal(self, shape):
        return jax.random.normal(self._next(), shape, dtype=jnp.bfloat16)
    def randint(self, lo, hi, shape):
        return jax.random.randint(self._next(), shape, lo, hi, dtype=jnp.int32)
    def uniform(self, shape, lo=0.0, hi=1.0):
        return jax.random.uniform(self._next(), shape, jnp.bfloat16, lo, hi)
    def permutation(self, n):
        return jax.random.permutation(self._next(), n)


kernel_name = 'standalone__mha_softmax__near_ridge'

def setup_inputs():
    _rng = _Rng(jax.random.key(int.from_bytes(__import__("os").urandom(4), "little")))
    _w = (lambda a: (lambda t: t.astype(jnp.bfloat16) if jnp.issubdtype(t.dtype, jnp.floating) else t)(jnp.asarray(a)))
    B, H, Sq, Sk, D = 32, 32, 288, 512, 128
    return {
        "q": _w((lambda *s: _rng.normal(s) * 0.4)(B, H, Sq, D)),
        "k": _w((lambda *s: _rng.normal(s) * 0.4)(B, H, Sk, D)),
        "v": _w((lambda *s: _rng.normal(s) * 0.05)(B, H, Sk, D)),
    }

def reference(q, k, v):
    scale = q.shape[-1] ** -0.5
    scores = jnp.einsum("bhqd,bhkd->bhqk", q, k) * scale
    p = _softmax(scores, axis=-1)
    return jnp.einsum("bhqk,bhkd->bhqd", p, v)
```

```python
import functools

import jax
import jax.numpy as jnp
from jax import lax
import jax.experimental.pallas as pl
import jax.experimental.pallas.tpu as pltpu

_LOG2E = 1.4426950408889634
_CHUNK = 8
_NBUF = 3


def _attend(q, k, v):
    c = (q.shape[-1] ** -0.5) * _LOG2E
    s = lax.dot_general(q, k, (((1,), (1,)), ((), ())),
                        preferred_element_type=jnp.float32)
    m = jnp.max(s, axis=-1, keepdims=True)
    p = jnp.exp2((s - m) * c)
    l = jnp.sum(p, axis=-1, keepdims=True)
    o = jnp.dot(p.astype(v.dtype), v, preferred_element_type=jnp.float32)
    return o * pl.reciprocal(l, approx=False, full_range=False)


def _mha_kernel(q_hbm, k_hbm, v_hbm, o_hbm, qb, kb, vb, ob, rsem, wsem):
    n = pl.num_programs(0)
    step = pl.program_id(0)
    bulk = o_hbm.shape[0] - _CHUNK

    def reads(chunk):
        slot = chunk % _NBUF
        return [
            pltpu.make_async_copy(src.at[pl.ds(chunk * _CHUNK, _CHUNK)],
                                  dst.at[slot], rsem.at[j, slot])
            for j, (src, dst) in enumerate(
                ((k_hbm, kb), (q_hbm, qb), (v_hbm, vb)))
        ]

    def write_bulk():
        return pltpu.make_async_copy(ob.at[pl.ds(0, bulk)],
                                     o_hbm.at[pl.ds(0, bulk)], wsem.at[0])

    def write_last():
        return pltpu.make_async_copy(ob.at[pl.ds(bulk, _CHUNK)],
                                     o_hbm.at[pl.ds(bulk, _CHUNK)], wsem.at[1])

    @pl.when(step == 0)
    def _():
        for chunk in range(_NBUF - 1):
            for cp in reads(chunk):
                cp.start()

    @pl.when(step + (_NBUF - 1) < n)
    def _():
        for cp in reads(step + (_NBUF - 1)):
            cp.start()

    for cp in reads(step):
        cp.wait()

    @pl.when(step == n - 1)
    def _():
        write_bulk().start()

    slot = step % _NBUF

    def body(g, carry):
        o = _attend(qb[slot, g], kb[slot, g], vb[slot, g])
        ob[step * _CHUNK + g] = o.astype(ob.dtype)
        return carry

    lax.fori_loop(0, _CHUNK, body, 0, unroll=True)

    @pl.when(step == n - 1)
    def _():
        write_last().start()
        write_bulk().wait()
        write_last().wait()


@jax.jit
def pallas_standalone__mha_softmax__near_ridge_kernel(
    q: jax.Array,
    k: jax.Array,
    v: jax.Array,
):
    b, h, sq, d = q.shape
    sk = k.shape[2]
    bh = b * h
    out = pl.pallas_call(
        _mha_kernel,
        grid=(bh // _CHUNK,),
        in_specs=[pl.BlockSpec(memory_space=pl.ANY)] * 3,
        out_specs=pl.BlockSpec(memory_space=pl.ANY),
        out_shape=jax.ShapeDtypeStruct((bh, sq, d), q.dtype),
        scratch_shapes=[
            pltpu.VMEM((_NBUF, _CHUNK, sq, d), q.dtype),
            pltpu.VMEM((_NBUF, _CHUNK, sk, d), k.dtype),
            pltpu.VMEM((_NBUF, _CHUNK, sk, d), v.dtype),
            pltpu.VMEM((bh, sq, d), q.dtype),
            pltpu.SemaphoreType.DMA((3, _NBUF)),
            pltpu.SemaphoreType.DMA((2,)),
        ],
        compiler_params=pltpu.CompilerParams(
            dimension_semantics=("arbitrary",),
            vmem_limit_bytes=110 * 1024 * 1024,
        ),
    )(q.reshape(bh, sq, d), k.reshape(bh, sk, d), v.reshape(bh, sk, d))
    return out.reshape(b, h, sq, d)
```

```python
import jax
import jax.numpy as jnp
from jax import lax
import jax.experimental.pallas as pl
import jax.experimental.pallas.tpu as pltpu

_LOG2E = 1.4426950408889634
_STREAMS = 8
_NBUF = 3
_WSPLIT = 2


def _attend(q, k, v):
    c = (q.shape[-1] ** -0.5) * _LOG2E
    s = lax.dot_general(q, k, (((1,), (1,)), ((), ())),
                        preferred_element_type=jnp.float32)
    m = jnp.max(s, axis=-1, keepdims=True)
    p = jnp.exp2((s - m) * c)
    l = jnp.sum(p, axis=-1, keepdims=True)
    o = jnp.dot(p.astype(v.dtype), v, preferred_element_type=jnp.float32)
    return o * pl.reciprocal(l, approx=False, full_range=False)


def _mha_kernel(q_hbm, k_hbm, v_hbm, o_hbm, qb, kb, vb, ob, rsem, wsem):
    n = pl.num_programs(0)
    step = pl.program_id(0)
    last = q_hbm.shape[1] - 1
    rows = q_hbm.shape[2] // _WSPLIT

    def reads(chunk):
        slot = chunk % _NBUF
        return [
            pltpu.make_async_copy(src.at[:, chunk], dst.at[slot],
                                  rsem.at[j, slot])
            for j, (src, dst) in enumerate(
                ((k_hbm, kb), (q_hbm, qb), (v_hbm, vb)))
        ]

    def start_writes(chunk):
        for j in range(_WSPLIT):
            sl = pl.ds(j * rows, rows)
            pltpu.make_async_copy(ob.at[chunk, :, sl], o_hbm.at[:, chunk, sl],
                                  wsem).start()

    @pl.when(step == 0)
    def _():
        for chunk in range(_NBUF - 1):
            for cp in reads(chunk):
                cp.start()

    @pl.when(step + (_NBUF - 1) < n)
    def _():
        for cp in reads(step + (_NBUF - 1)):
            cp.start()

    for cp in reads(step):
        cp.wait()

    @pl.when(step == n - 1)
    def _():
        def issue(chunk, carry):
            start_writes(chunk)
            return carry

        lax.fori_loop(0, last, issue, 0)

    slot = step % _NBUF

    def body(g, carry):
        o = _attend(qb[slot, g], kb[slot, g], vb[slot, g])
        ob[step, g] = o.astype(ob.dtype)
        return carry

    lax.fori_loop(0, _STREAMS, body, 0, unroll=True)

    @pl.when(step == n - 1)
    def _():
        start_writes(last)
        pltpu.make_async_copy(ob, ob, wsem).wait()


@jax.jit
def pallas_standalone__mha_softmax__near_ridge_kernel(
    q: jax.Array,
    k: jax.Array,
    v: jax.Array,
):
    b, h, sq, d = q.shape
    sk = k.shape[2]
    n = (b * h) // _STREAMS
    out = pl.pallas_call(
        _mha_kernel,
        grid=(n,),
        in_specs=[pl.BlockSpec(memory_space=pl.ANY)] * 3,
        out_specs=pl.BlockSpec(memory_space=pl.ANY),
        out_shape=jax.ShapeDtypeStruct((_STREAMS, n, sq, d), q.dtype),
        scratch_shapes=[
            pltpu.VMEM((_NBUF, _STREAMS, sq, d), q.dtype),
            pltpu.VMEM((_NBUF, _STREAMS, sk, d), k.dtype),
            pltpu.VMEM((_NBUF, _STREAMS, sk, d), v.dtype),
            pltpu.VMEM((n, _STREAMS, sq, d), q.dtype),
            pltpu.SemaphoreType.DMA((3, _NBUF)),
            pltpu.SemaphoreType.DMA(()),
        ],
        compiler_params=pltpu.CompilerParams(
            dimension_semantics=("arbitrary",),
            vmem_limit_bytes=110 * 1024 * 1024,
        ),
    )(
        q.reshape(_STREAMS, n, sq, d),
        k.reshape(_STREAMS, n, sk, d),
        v.reshape(_STREAMS, n, sk, d),
    )
    return out.reshape(b, h, sq, d)
```

```python
import jax
import jax.numpy as jnp
from jax import lax
import jax.experimental.pallas as pl
import jax.experimental.pallas.tpu as pltpu

_LOG2E = 1.4426950408889634
_STREAMS = 8
_NBUF = 3
_WSPLIT = 2
_WFIRST = 32


def _attend(q, k, v):
    c = (q.shape[-1] ** -0.5) * _LOG2E
    s = lax.dot_general(q, k, (((1,), (1,)), ((), ())),
                        preferred_element_type=jnp.float32)
    m = jnp.max(s, axis=-1, keepdims=True)
    p = jnp.exp2((s - m) * c)
    l = jnp.sum(p, axis=-1, keepdims=True)
    o = jnp.dot(p.astype(v.dtype), v, preferred_element_type=jnp.float32)
    return o * pl.reciprocal(l, approx=False, full_range=False)


def _mha_kernel(q_hbm, k_hbm, v_hbm, o_hbm, qb, kb, vb, ob, stage,
                rsem, hsem, ssem, wsem):
    n = q_hbm.shape[1]
    step = pl.program_id(0)
    rows = q_hbm.shape[2] // _WSPLIT
    side = _STREAMS - 1

    def reads(t):
        slot = t % _NBUF
        return [
            pltpu.make_async_copy(k_hbm.at[:, t], kb.at[slot],
                                  rsem.at[0, slot]),
            pltpu.make_async_copy(v_hbm.at[:, t], vb.at[slot],
                                  rsem.at[1, slot]),
            pltpu.make_async_copy(q_hbm.at[pl.ds(0, side), t],
                                  qb.at[slot, pl.ds(0, side)],
                                  rsem.at[2, slot]),
        ]

    def to_smem(t):
        return pltpu.make_async_copy(q_hbm.at[side, t], stage.at[t % 2],
                                     hsem.at[t % 2])

    def from_smem(t):
        return pltpu.make_async_copy(stage.at[t % 2], qb.at[t % _NBUF, side],
                                     ssem.at[t % _NBUF])

    def start_writes(t, carry):
        for j in range(_WSPLIT):
            sl = pl.ds(j * rows, rows)
            pltpu.make_async_copy(ob.at[t, :, sl], o_hbm.at[:, t, sl],
                                  wsem).start()
        return carry

    @pl.when(step == 0)
    def _():
        for cp in reads(0):
            cp.start()
        pltpu.make_async_copy(q_hbm.at[side, 0], qb.at[0, side],
                              ssem.at[0]).start()
        for t in range(1, _NBUF - 1):
            for cp in reads(t):
                cp.start()
        to_smem(1).start()

    @pl.when(step + (_NBUF - 1) < n)
    def _():
        for cp in reads(step + (_NBUF - 1)):
            cp.start()

    @pl.when(step + 1 < n)
    def _():
        to_smem(step + 1).wait()
        from_smem(step + 1).start()

    from_smem(step).wait()

    @pl.when(step + 2 < n)
    def _():
        to_smem(step + 2).start()

    k_copy, v_copy, q_copy = reads(step)
    k_copy.wait()
    v_copy.wait()

    @pl.when(step == n - 1)
    def _():
        lax.fori_loop(0, _WFIRST, start_writes, 0)

    q_copy.wait()

    slot = step % _NBUF
    for g in range(_STREAMS):
        o = _attend(qb[slot, g], kb[slot, g], vb[slot, g])
        ob[step, g] = o.astype(ob.dtype)

    @pl.when(step == n - 1)
    def _():
        lax.fori_loop(_WFIRST, n, start_writes, 0)
        pltpu.make_async_copy(ob, ob, wsem).wait()


@jax.jit
def pallas_standalone__mha_softmax__near_ridge_kernel(
    q: jax.Array,
    k: jax.Array,
    v: jax.Array,
):
    b, h, sq, d = q.shape
    sk = k.shape[2]
    n = (b * h) // _STREAMS
    out = pl.pallas_call(
        _mha_kernel,
        grid=(n,),
        in_specs=[pl.BlockSpec(memory_space=pl.ANY)] * 3,
        out_specs=pl.BlockSpec(memory_space=pl.ANY),
        out_shape=jax.ShapeDtypeStruct((_STREAMS, n, sq, d), q.dtype),
        scratch_shapes=[
            pltpu.VMEM((_NBUF, _STREAMS, sq, d), q.dtype),
            pltpu.VMEM((_NBUF, _STREAMS, sk, d), k.dtype),
            pltpu.VMEM((_NBUF, _STREAMS, sk, d), v.dtype),
            pltpu.VMEM((n, _STREAMS, sq, d), q.dtype),
            pltpu.SMEM((2, sq, d), q.dtype),
            pltpu.SemaphoreType.DMA((3, _NBUF)),
            pltpu.SemaphoreType.DMA((2,)),
            pltpu.SemaphoreType.DMA((_NBUF,)),
            pltpu.SemaphoreType.DMA(()),
        ],
        compiler_params=pltpu.CompilerParams(
            dimension_semantics=("arbitrary",),
            vmem_limit_bytes=110 * 1024 * 1024,
        ),
    )(
        q.reshape(_STREAMS, n, sq, d),
        k.reshape(_STREAMS, n, sk, d),
        v.reshape(_STREAMS, n, sk, d),
    )
    return out.reshape(b, h, sq, d)
```

```python
import jax
import jax.numpy as jnp
from jax import lax
import jax.experimental.pallas as pl
import jax.experimental.pallas.tpu as pltpu

_LOG2E = 1.4426950408889634

_HEADS = 8
_NBUF = 3
_K_SPLIT = (256, 256)
_V_SPLIT = (192, 160, 160)
_SIDE = (48, 32, 48, 32, 48, 32, 48, 32)
_LAG = 2
_W_STREAMS = 9
_W_ROWS = 144
_W_FIRST = 26


def _attend(q, k, v):
    c = (q.shape[-1] ** -0.5) * _LOG2E
    s = lax.dot_general(q, k, (((1,), (1,)), ((), ())),
                        preferred_element_type=jnp.float32)
    m = jnp.max(s, axis=-1, keepdims=True)
    p = jnp.exp2((s - m) * c)
    l = jnp.sum(p, axis=-1, keepdims=True)
    o = jnp.dot(p.astype(v.dtype), v, preferred_element_type=jnp.float32)
    return o * pl.reciprocal(l, approx=False, full_range=False)


def _mha_kernel(q_hbm, k_hbm, v_hbm, o_hbm, qb, kb, vb, ob, stage,
                rsem, hsem, ssem, wsem):
    _, n, sq, _ = q_hbm.shape
    sk = k_hbm.shape[2]
    step = pl.program_id(0)
    last = _HEADS - 1
    nstage = 2 * _LAG
    side_rows = sum(_SIDE)
    side0 = sk - side_rows
    w_len = o_hbm.shape[0] // _W_STREAMS
    w_cols = w_len // _W_ROWS

    def reads(t):
        slot = t % _NBUF
        parts = []
        for src, dst, split in ((k_hbm, kb, _K_SPLIT), (v_hbm, vb, _V_SPLIT),
                                (q_hbm, qb, (sq,))):
            r0 = 0
            for rows in split:
                heads = last if (src is v_hbm and r0 >= side0) else _HEADS
                parts.append(
                    (src.at[pl.ds(0, heads), t, pl.ds(r0, rows)],
                     dst.at[slot, pl.ds(0, heads), pl.ds(r0, rows)]))
                r0 += rows
        return [pltpu.make_async_copy(src, dst, rsem.at[j, slot])
                for j, (src, dst) in enumerate(parts)]

    def to_smem(t, off, rows):
        return pltpu.make_async_copy(
            v_hbm.at[last, t, pl.ds(side0 + off, rows)],
            stage.at[t % nstage, pl.ds(off, rows)], hsem.at[t % nstage])

    def from_smem(t, off, rows):
        return pltpu.make_async_copy(
            stage.at[t % nstage, pl.ds(off, rows)],
            vb.at[t % _NBUF, last, pl.ds(side0 + off, rows)],
            ssem.at[t % _NBUF])

    def start_side(g):
        off, rows = sum(_SIDE[:g]), _SIDE[g]

        @pl.when(step + nstage < n)
        def _():
            to_smem(step + nstage, off, rows).start()

        @pl.when(step + _LAG < n)
        def _():
            from_smem(step + _LAG, off, rows).start()

    def start_write(r0, rows):
        for u in range(_W_STREAMS):
            sl = pl.ds(pl.multiple_of(u * w_len + r0, 16), rows)
            pltpu.make_async_copy(ob.at[sl], o_hbm.at[sl], wsem).start()

    def write_loop(j, carry):
        start_write(j * _W_ROWS, _W_ROWS)
        return carry

    @pl.when(step == 0)
    def _():
        for t in range(_NBUF - 1):
            for cp in reads(t):
                cp.start()
            pltpu.make_async_copy(
                v_hbm.at[last, t, pl.ds(side0, side_rows)],
                vb.at[t, last, pl.ds(side0, side_rows)], ssem.at[t]).start()
        for t in range(_LAG, nstage):
            to_smem(t, 0, side_rows).start()

    @pl.when(step + (_NBUF - 1) < n)
    def _():
        for cp in reads(step + (_NBUF - 1)):
            cp.start()

    @pl.when(step + _LAG < n)
    def _():
        to_smem(step + _LAG, 0, side_rows).wait()

    from_smem(step, 0, side_rows).wait()
    start_side(0)

    copies = reads(step)
    for cp in copies[:-1]:
        cp.wait()

    @pl.when(step == n - 1)
    def _():
        lax.fori_loop(0, _W_FIRST, write_loop, 0)

    copies[-1].wait()

    slot = step % _NBUF
    for g in range(_HEADS):
        if g:
            start_side(g)
        o = _attend(qb[slot, g], kb[slot, g], vb[slot, g])
        row = pl.multiple_of((g * n + step) * sq, 16)
        ob[pl.ds(row, sq), :] = o.astype(ob.dtype)

    @pl.when(step == n - 1)
    def _():
        lax.fori_loop(_W_FIRST, w_cols, write_loop, 0)
        start_write(w_cols * _W_ROWS, w_len - w_cols * _W_ROWS)
        pltpu.make_async_copy(ob, o_hbm, wsem).wait()


@jax.jit
def pallas_standalone__mha_softmax__near_ridge_kernel(
    q: jax.Array,
    k: jax.Array,
    v: jax.Array,
):
    b, h, sq, d = q.shape
    sk = k.shape[2]
    n = (b * h) // _HEADS
    rows = b * h * sq
    w_len = rows // _W_STREAMS
    assert _LAG == _NBUF - 1 and len(_SIDE) == _HEADS
    assert sum(_K_SPLIT) == sk and sum(_V_SPLIT) == sk
    assert _V_SPLIT[0] == sk - sum(_SIDE)
    assert rows % _W_STREAMS == 0 and w_len % _W_ROWS != 0
    assert all(((g * n + n - 1) * sq + r) % w_len >= _W_FIRST * _W_ROWS
               for g in range(_HEADS) for r in range(sq))
    out = pl.pallas_call(
        _mha_kernel,
        grid=(n,),
        in_specs=[pl.BlockSpec(memory_space=pl.ANY)] * 3,
        out_specs=pl.BlockSpec(memory_space=pl.ANY),
        out_shape=jax.ShapeDtypeStruct((rows, d), q.dtype),
        scratch_shapes=[
            pltpu.VMEM((_NBUF, _HEADS, sq, d), q.dtype),
            pltpu.VMEM((_NBUF, _HEADS, sk, d), k.dtype),
            pltpu.VMEM((_NBUF, _HEADS, sk, d), v.dtype),
            pltpu.VMEM((rows, d), q.dtype),
            pltpu.SMEM((2 * _LAG, sum(_SIDE), d), v.dtype),
            pltpu.SemaphoreType.DMA(
                (len(_K_SPLIT) + len(_V_SPLIT) + 1, _NBUF)),
            pltpu.SemaphoreType.DMA((2 * _LAG,)),
            pltpu.SemaphoreType.DMA((_NBUF,)),
            pltpu.SemaphoreType.DMA(()),
        ],
        compiler_params=pltpu.CompilerParams(
            dimension_semantics=("arbitrary",),
            vmem_limit_bytes=110 * 1024 * 1024,
            disable_bounds_checks=True,
        ),
    )(
        q.reshape(_HEADS, n, sq, d),
        k.reshape(_HEADS, n, sk, d),
        v.reshape(_HEADS, n, sk, d),
    )
    return out.reshape(b, h, sq, d)
```

```python
import jax
import jax.numpy as jnp
from jax import lax
import jax.experimental.pallas as pl
import jax.experimental.pallas.tpu as pltpu

_LOG2E = 1.4426950408889634

_HEADS = 8
_NBUF = 3
_K_SPLIT = (256, 256)
_V_SPLIT = (192, 160, 160)
_SIDE = (48, 32, 48, 32, 48, 32, 48, 32)
_LAG = 2
_W_STREAMS = 9
_W_ROWS = 112
_W_EARLY = (7, 208)


def _attend(q, k, v):
    c = (q.shape[-1] ** -0.5) * _LOG2E
    s = lax.dot_general(q, k, (((1,), (1,)), ((), ())),
                        preferred_element_type=jnp.float32)
    m = jnp.max(s, axis=-1, keepdims=True)
    p = jnp.exp2((s - m) * c)
    l = jnp.sum(p, axis=-1, keepdims=True)
    o = jnp.dot(p.astype(v.dtype), v, preferred_element_type=jnp.float32)
    return o * pl.reciprocal(l, approx=False, full_range=False)


def _mha_kernel(q_hbm, k_hbm, v_hbm, o_hbm, qb, kb, vb, ob, stage,
                rsem, hsem, ssem, wsem):
    _, n, sq, _ = q_hbm.shape
    sk = k_hbm.shape[2]
    step = pl.program_id(0)
    last = _HEADS - 1
    nstage = 2 * _LAG
    side_rows = sum(_SIDE)
    side0 = sk - side_rows
    w_len = o_hbm.shape[0] // _W_STREAMS
    w_base = _W_EARLY[0] * _W_EARLY[1]
    w_cols = (w_len - w_base) // _W_ROWS
    w_tail = w_base + w_cols * _W_ROWS

    def reads(t):
        slot = t % _NBUF
        parts = []
        for src, dst, split in ((k_hbm, kb, _K_SPLIT), (v_hbm, vb, _V_SPLIT),
                                (q_hbm, qb, (sq,))):
            r0 = 0
            for rows in split:
                heads = last if (src is v_hbm and r0 >= side0) else _HEADS
                parts.append(
                    (src.at[pl.ds(0, heads), t, pl.ds(r0, rows)],
                     dst.at[slot, pl.ds(0, heads), pl.ds(r0, rows)]))
                r0 += rows
        return [pltpu.make_async_copy(src, dst, rsem.at[j, slot])
                for j, (src, dst) in enumerate(parts)]

    def to_smem(t, off, rows):
        return pltpu.make_async_copy(
            v_hbm.at[last, t, pl.ds(side0 + off, rows)],
            stage.at[t % nstage, pl.ds(off, rows)], hsem.at[t % nstage])

    def from_smem(t, off, rows):
        return pltpu.make_async_copy(
            stage.at[t % nstage, pl.ds(off, rows)],
            vb.at[t % _NBUF, last, pl.ds(side0 + off, rows)],
            ssem.at[t % _NBUF])

    def start_side(g):
        off, rows = sum(_SIDE[:g]), _SIDE[g]

        @pl.when(step + nstage < n)
        def _():
            to_smem(step + nstage, off, rows).start()

        @pl.when(step + _LAG < n)
        def _():
            from_smem(step + _LAG, off, rows).start()

    def start_write(r0, rows):
        for u in range(_W_STREAMS):
            sl = pl.ds(pl.multiple_of(u * w_len + r0, 16), rows)
            pltpu.make_async_copy(ob.at[sl], o_hbm.at[sl], wsem).start()

    def early_writes(j, carry):
        start_write(j * _W_EARLY[1], _W_EARLY[1])
        return carry

    def late_writes(j, carry):
        start_write(w_base + j * _W_ROWS, _W_ROWS)
        return carry

    @pl.when(step == 0)
    def _():
        for t in range(_NBUF - 1):
            for cp in reads(t):
                cp.start()
            pltpu.make_async_copy(
                v_hbm.at[last, t, pl.ds(side0, side_rows)],
                vb.at[t, last, pl.ds(side0, side_rows)], ssem.at[t]).start()
        for t in range(_LAG, nstage):
            to_smem(t, 0, side_rows).start()

    @pl.when(step + (_NBUF - 1) < n)
    def _():
        for cp in reads(step + (_NBUF - 1)):
            cp.start()

    @pl.when(step + _LAG < n)
    def _():
        to_smem(step + _LAG, 0, side_rows).wait()

    from_smem(step, 0, side_rows).wait()
    start_side(0)

    copies = reads(step)
    for cp in copies[:-1]:
        cp.wait()

    @pl.when(step == n - 1)
    def _():
        lax.fori_loop(0, _W_EARLY[0], early_writes, 0)

    copies[-1].wait()

    slot = step % _NBUF
    for g in range(_HEADS):
        if g:
            start_side(g)
        o = _attend(qb[slot, g], kb[slot, g], vb[slot, g])
        row = pl.multiple_of((g * n + step) * sq, 16)
        ob[pl.ds(row, sq), :] = o.astype(ob.dtype)

    @pl.when(step == n - 1)
    def _():
        lax.fori_loop(0, w_cols, late_writes, 0)
        if w_tail < w_len:
            start_write(w_tail, w_len - w_tail)
        pltpu.make_async_copy(ob, o_hbm, wsem).wait()


@jax.jit
def pallas_standalone__mha_softmax__near_ridge_kernel(
    q: jax.Array,
    k: jax.Array,
    v: jax.Array,
):
    b, h, sq, d = q.shape
    sk = k.shape[2]
    n = (b * h) // _HEADS
    rows = b * h * sq
    w_len = rows // _W_STREAMS
    assert _LAG == _NBUF - 1 and len(_SIDE) == _HEADS
    assert sum(_K_SPLIT) == sk and sum(_V_SPLIT) == sk
    assert _V_SPLIT[0] == sk - sum(_SIDE)
    assert rows % _W_STREAMS == 0 and w_len % 16 == 0
    assert all(((g * n + n - 1) * sq + r) % w_len >= _W_EARLY[0] * _W_EARLY[1]
               for g in range(_HEADS) for r in range(sq))
    out = pl.pallas_call(
        _mha_kernel,
        grid=(n,),
        in_specs=[pl.BlockSpec(memory_space=pl.ANY)] * 3,
        out_specs=pl.BlockSpec(memory_space=pl.ANY),
        out_shape=jax.ShapeDtypeStruct((rows, d), q.dtype),
        scratch_shapes=[
            pltpu.VMEM((_NBUF, _HEADS, sq, d), q.dtype),
            pltpu.VMEM((_NBUF, _HEADS, sk, d), k.dtype),
            pltpu.VMEM((_NBUF, _HEADS, sk, d), v.dtype),
            pltpu.VMEM((rows, d), q.dtype),
            pltpu.SMEM((2 * _LAG, sum(_SIDE), d), v.dtype),
            pltpu.SemaphoreType.DMA(
                (len(_K_SPLIT) + len(_V_SPLIT) + 1, _NBUF)),
            pltpu.SemaphoreType.DMA((2 * _LAG,)),
            pltpu.SemaphoreType.DMA((_NBUF,)),
            pltpu.SemaphoreType.DMA(()),
        ],
        compiler_params=pltpu.CompilerParams(
            dimension_semantics=("arbitrary",),
            vmem_limit_bytes=110 * 1024 * 1024,
            disable_bounds_checks=True,
        ),
    )(
        q.reshape(_HEADS, n, sq, d),
        k.reshape(_HEADS, n, sk, d),
        v.reshape(_HEADS, n, sk, d),
    )
    return out.reshape(b, h, sq, d)
```

```python
import jax
import jax.numpy as jnp
from jax import lax
import jax.experimental.pallas as pl
import jax.experimental.pallas.tpu as pltpu

_LOG2E = 1.4426950408889634

_HEADS = 8
_NBUF = 3
_K_SPLIT = (256, 256)
_V_SPLIT = (192, 160, 160)
_SIDE = (48, 32, 48, 32, 48, 32, 48, 32)
_LAG = 2
_W_STREAMS = 9
_W_ROWS = 112
_W_EARLY = (7, 208)


def _attend(q, k, v):
    c = (q.shape[-1] ** -0.5) * _LOG2E
    s = lax.dot_general(q, k, (((1,), (1,)), ((), ())),
                        preferred_element_type=jnp.float32)
    m = jnp.max(s, axis=-1, keepdims=True)
    p = jnp.exp2((s - m) * c)
    l = jnp.sum(p, axis=-1, keepdims=True)
    o = jnp.dot(p.astype(v.dtype), v, preferred_element_type=jnp.float32)
    return o * pl.reciprocal(l, approx=False, full_range=False)


def _mha_kernel(q_hbm, k_hbm, v_hbm, o_hbm, qb, kb, vb, ob, stage,
                rsem, hsem, ssem, wsem):
    _, n, sq, _ = q_hbm.shape
    sk = k_hbm.shape[2]
    step = pl.program_id(0)
    last = _HEADS - 1
    nstage = 2 * _LAG
    side_rows = sum(_SIDE)
    side0 = sk - side_rows
    w_len = o_hbm.shape[0] // _W_STREAMS
    w_base = _W_EARLY[0] * _W_EARLY[1]
    w_cols = (w_len - w_base) // _W_ROWS
    w_tail = w_base + w_cols * _W_ROWS

    def reads(t):
        slot = t % _NBUF
        parts = []
        for src, dst, split in ((k_hbm, kb, _K_SPLIT), (v_hbm, vb, _V_SPLIT),
                                (q_hbm, qb, (sq,))):
            r0 = 0
            for rows in split:
                heads = last if (src is v_hbm and r0 >= side0) else _HEADS
                parts.append(
                    (src.at[pl.ds(0, heads), t, pl.ds(r0, rows)],
                     dst.at[slot, pl.ds(0, heads), pl.ds(r0, rows)]))
                r0 += rows
        return [pltpu.make_async_copy(src, dst, rsem.at[j, slot])
                for j, (src, dst) in enumerate(parts)]

    def to_smem(t, off, rows):
        return pltpu.make_async_copy(
            v_hbm.at[last, t, pl.ds(side0 + off, rows)],
            stage.at[t % nstage, pl.ds(off, rows)], hsem.at[t % nstage])

    def from_smem(t, off, rows):
        return pltpu.make_async_copy(
            stage.at[t % nstage, pl.ds(off, rows)],
            vb.at[t % _NBUF, last, pl.ds(side0 + off, rows)],
            ssem.at[t % _NBUF])

    def direct(t):
        return pltpu.make_async_copy(
            v_hbm.at[last, t, pl.ds(side0, side_rows)],
            vb.at[t % _NBUF, last, pl.ds(side0, side_rows)],
            ssem.at[t % _NBUF])

    def start_side(g):
        off, rows = sum(_SIDE[:g]), _SIDE[g]

        @pl.when(step + nstage < n)
        def _():
            to_smem(step + nstage, off, rows).start()

        @pl.when(step + _LAG < n)
        def _():
            from_smem(step + _LAG, off, rows).start()

    def start_write(r0, rows):
        for u in range(_W_STREAMS):
            sl = pl.ds(pl.multiple_of(u * w_len + r0, 16), rows)
            pltpu.make_async_copy(ob.at[sl], o_hbm.at[sl], wsem).start()

    def early_writes(j, carry):
        start_write(j * _W_EARLY[1], _W_EARLY[1])
        return carry

    def late_writes(j, carry):
        start_write(w_base + j * _W_ROWS, _W_ROWS)
        return carry

    @pl.when(step == 0)
    def _():
        for t in range(_NBUF - 1):
            for cp in reads(t):
                cp.start()
            direct(t).start()
        for t in range(_LAG, nstage):
            to_smem(t, 0, side_rows).start()

    @pl.when(step + (_NBUF - 1) < n)
    def _():
        for cp in reads(step + (_NBUF - 1)):
            cp.start()

    @pl.when(step + _LAG < n)
    def _():
        to_smem(step + _LAG, 0, side_rows).wait()

    @pl.when(step < _LAG)
    def _():
        direct(step).wait()

    @pl.when(step >= _LAG)
    def _():
        from_smem(step, 0, side_rows).wait()

    start_side(0)

    copies = reads(step)
    for cp in copies[:-1]:
        cp.wait()

    @pl.when(step == n - 1)
    def _():
        lax.fori_loop(0, _W_EARLY[0], early_writes, 0)

    copies[-1].wait()

    slot = step % _NBUF
    for g in range(_HEADS):
        if g:
            start_side(g)
        o = _attend(qb[slot, g], kb[slot, g], vb[slot, g])
        row = pl.multiple_of((g * n + step) * sq, 16)
        ob[pl.ds(row, sq), :] = o.astype(ob.dtype)

    @pl.when(step == n - 1)
    def _():
        lax.fori_loop(0, w_cols, late_writes, 0)
        if w_tail < w_len:
            start_write(w_tail, w_len - w_tail)
        pltpu.make_async_copy(ob, o_hbm, wsem).wait()


@jax.jit
def pallas_standalone__mha_softmax__near_ridge_kernel(
    q: jax.Array,
    k: jax.Array,
    v: jax.Array,
):
    b, h, sq, d = q.shape
    sk = k.shape[2]
    n = (b * h) // _HEADS
    rows = b * h * sq
    w_len = rows // _W_STREAMS
    assert _LAG == _NBUF - 1 and len(_SIDE) == _HEADS
    assert sum(_K_SPLIT) == sk and sum(_V_SPLIT) == sk
    assert _V_SPLIT[0] == sk - sum(_SIDE)
    assert rows % _W_STREAMS == 0 and w_len % 16 == 0
    assert all(((g * n + n - 1) * sq + r) % w_len >= _W_EARLY[0] * _W_EARLY[1]
               for g in range(_HEADS) for r in range(sq))
    out = pl.pallas_call(
        _mha_kernel,
        grid=(n,),
        in_specs=[pl.BlockSpec(memory_space=pl.ANY)] * 3,
        out_specs=pl.BlockSpec(memory_space=pl.ANY),
        out_shape=jax.ShapeDtypeStruct((rows, d), q.dtype),
        scratch_shapes=[
            pltpu.VMEM((_NBUF, _HEADS, sq, d), q.dtype),
            pltpu.VMEM((_NBUF, _HEADS, sk, d), k.dtype),
            pltpu.VMEM((_NBUF, _HEADS, sk, d), v.dtype),
            pltpu.VMEM((rows, d), q.dtype),
            pltpu.SMEM((2 * _LAG, sum(_SIDE), d), v.dtype),
            pltpu.SemaphoreType.DMA(
                (len(_K_SPLIT) + len(_V_SPLIT) + 1, _NBUF)),
            pltpu.SemaphoreType.DMA((2 * _LAG,)),
            pltpu.SemaphoreType.DMA((_NBUF,)),
            pltpu.SemaphoreType.DMA(()),
        ],
        compiler_params=pltpu.CompilerParams(
            dimension_semantics=("arbitrary",),
            vmem_limit_bytes=110 * 1024 * 1024,
            disable_bounds_checks=True,
        ),
    )(
        q.reshape(_HEADS, n, sq, d),
        k.reshape(_HEADS, n, sk, d),
        v.reshape(_HEADS, n, sk, d),
    )
    return out.reshape(b, h, sq, d)
```
